```python
import jax
import jax.numpy as jnp

def _softmax(x, axis=-1):
    return jax.nn.softmax(x, axis=axis)
def _gelu(x):
    return jax.nn.gelu(x, approximate=True)
def _silu(x):
    return jax.nn.silu(x)
def _sigmoid(x):
    return jax.nn.sigmoid(x)
def _layernorm(x, axis=-1, eps=1e-5):
    m = jnp.mean(x, axis=axis, keepdims=True)
    v = jnp.var(x, axis=axis, keepdims=True)
    return (x - m) / jnp.sqrt(v + eps)
def _scatter_add(tgt, idx, src, axis=0):
    return tgt.at[idx].add(src)
def _segment_sum(src, seg, n):
    return jax.ops.segment_sum(src, seg, n)
class _Rng:
    def __init__(self, key):
        self._k = key
    def _next(self):
        self._k, sub = jax.random.split(self._k)
        return sub
    def normal(self, shape):
        return jax.random.normal(self._next(), shape, dtype=jnp.bfloat16)
    def randint(self, lo, hi, shape):
        return jax.random.randint(self._next(), shape, lo, hi, dtype=jnp.int32)
    def uniform(self, shape, lo=0.0, hi=1.0):
        return jax.random.uniform(self._next(), shape, jnp.bfloat16, lo, hi)
    def permutation(self, n):
        return jax.random.permutation(self._next(), n)


kernel_name = 'interleave_layers__sliding_local_dilated__mixer_token_mlp__prompt'

def setup_inputs():
    _rng = _Rng(jax.random.key(int.from_bytes(__import__("os").urandom(4), "little")))
    _w = (lambda a: (lambda t: t.astype(jnp.bfloat16) if jnp.issubdtype(t.dtype, jnp.floating) else t)(jnp.asarray(a)))
    def _A_setup():
        B, S, D = 1, 2048, 1024
        return {
            "x": _w((lambda *s: _rng.normal(s) * 0.05)(B, S, D)),
            "wqkv": _w((lambda *s: _rng.normal(s) * 0.05)(D, 3 * D)),
            "wo": _w((lambda *s: _rng.normal(s) * 0.05)(D, D)),
        }
    _A_in = _A_setup()

    def _B_setup():
        B, S, D, F = 1, 2048, 1024, 3584
        return {
            "x": _w((lambda *s: _rng.normal(s) * 0.05)(B, S, D)),
            "w1": _w((lambda *s: _rng.normal(s) * 0.05)(S, F) * (S ** -0.5)),
            "b1": _w((lambda *s: _rng.normal(s) * 0.05)(F) * 0.02),
            "w2": _w((lambda *s: _rng.normal(s) * 0.05)(F, S) * (F ** -0.5)),
            "b2": _w((lambda *s: _rng.normal(s) * 0.05)(S) * 0.02),
        }
    _B_in = _B_setup()

    return {
        "A_x": _A_in["x"],
        "A_wqkv": _A_in["wqkv"],
        "A_wo": _A_in["wo"],
        "B_x": _B_in["x"],
        "B_w1": _B_in["w1"],
        "B_b1": _B_in["b1"],
        "B_w2": _B_in["w2"],
        "B_b2": _B_in["b2"],
    }

def reference(A_x, A_wqkv, A_wo, B_x, B_w1, B_b1, B_w2, B_b2):
    def _A_ref(x, wqkv, wo):
        B, S, D = x.shape
        H = 32; Dh = D // H
        W, dil = 8, 2
        qkv = (lambda x, *d: x.transpose(*d))((x @ wqkv).reshape(B, S, 3, H, Dh), 2, 0, 3, 1, 4)
        q, k, v = qkv[0], qkv[1], qkv[2]
        scale = Dh ** -0.5
        pos = jnp.arange(S)
        off = jnp.arange(W) * dil
        idx = pos[:, None] - off[None, :]
        mask = idx >= 0
        idx_c = jnp.where(mask, idx, 0).reshape(-1)
        kg = k[:, :, idx_c, :].reshape(B, H, S, W, Dh)
        vg = v[:, :, idx_c, :].reshape(B, H, S, W, Dh)
        logits = jnp.einsum("bhsd,bhswd->bhsw", q, kg) * scale
        logits = jnp.where(mask[None, None, :, :], logits, -1e9)
        attn = _softmax(logits, axis=-1)
        o = jnp.einsum("bhsw,bhswd->bhsd", attn, vg)
        return (lambda x, *d: x.transpose(*d))(o, 0, 2, 1, 3).reshape(B, S, D) @ wo

    def _B_ref(x, w1, b1, w2, b2):
        B, S, D = x.shape
        h = _layernorm(x, axis=-1)
        u = jnp.einsum("bsd,sf->bdf", h, w1) + b1
        u = _gelu(u)
        y = jnp.einsum("bdf,fs->bds", u, w2) + b2
        return (lambda x, *d: x.transpose(*d))(y, 0, 2, 1)

    x = A_x
    x = x + _A_ref(_layernorm(x, axis=-1), A_wqkv, A_wo)
    x = x + _B_ref(_layernorm(x, axis=-1), B_w1, B_b1, B_w2, B_b2)
    x = x + _A_ref(_layernorm(x, axis=-1), A_wqkv, A_wo)
    x = x + _B_ref(_layernorm(x, axis=-1), B_w1, B_b1, B_w2, B_b2)
    return x
```

```python
import jax
import jax.numpy as jnp
import numpy as np
import jax.experimental.pallas as pl
import jax.experimental.pallas.tpu as pltpu

S, D, F = 2048, 1024, 3584
H, DH, W, DIL = 32, 32, 8, 2
EPS = 1e-5
PAD = 16
TA = 256
TF = 512
TS = 256
NB = D // 128
f32, bf16 = jnp.float32, jnp.bfloat16


def _dot(a, b):
    return jnp.dot(a, b, preferred_element_type=f32)


def _ln_stats(x):
    m = jnp.mean(x, axis=-1, keepdims=True)
    xc = x - m
    v = jnp.mean(xc * xc, axis=-1, keepdims=True)
    return xc, v


def _head_minor_rows(tmp):
    return jnp.concatenate(
        [tmp[pl.ds(c, H, stride=DH), :] for c in range(DH)], axis=0)


def _kernel(x_hbm, wqkv_hbm, wo_hbm, w1_hbm, b1_ref, w2_hbm, b2_ref, out_hbm,
            xin, wqkv, wo, w1, w2, xs, tmpu, tmpf, q_s, k_s, v_s, o_s, ht, g_s,
            sems):
    cp_x = pltpu.make_async_copy(x_hbm, xin, sems.at[0])
    cp_qkv = pltpu.make_async_copy(wqkv_hbm, wqkv, sems.at[1])
    cp_wo = pltpu.make_async_copy(wo_hbm, wo, sems.at[2])
    cp_w1 = pltpu.make_async_copy(w1_hbm, w1, sems.at[3])
    cp_w2 = pltpu.make_async_copy(w2_hbm, w2, sems.at[4])
    cp_qkv.start()
    cp_x.start()
    cp_wo.start()
    cp_w1.start()
    cp_w2.start()

    cp_qkv.wait()

    def perm_qkv(i, _):
        r = pl.multiple_of((i // 3) * 256, 256)
        c = pl.multiple_of((i % 3) * D, D)
        blk = pltpu.bitcast(wqkv[pl.ds(r, 256), pl.ds(c, D)], jnp.uint32)
        tmpu[...] = blk.T
        wqkv[pl.ds(r, 256), pl.ds(c, D)] = pltpu.bitcast(
            _head_minor_rows(tmpu).T, bf16)
        return 0
    jax.lax.fori_loop(0, 12, perm_qkv, 0)

    cp_wo.wait()

    def perm_wo(i, _):
        c = pl.multiple_of(i * 128, 128)
        tmpf[...] = wo[:, pl.ds(c, 128)].astype(f32)
        wo[:, pl.ds(c, 128)] = _head_minor_rows(tmpf).astype(bf16)
        return 0
    jax.lax.fori_loop(0, NB, perm_wo, 0)

    cp_x.wait()
    xs[...] = xin[...].astype(f32)

    def attn_block(i, _):
        r0 = pl.multiple_of(i * TA, TA)
        xc, var = _ln_stats(xs[pl.ds(r0, TA), :])
        ln = (xc * jax.lax.rsqrt(var + EPS)).astype(bf16)
        qkv = _dot(ln, wqkv[...])
        for b in range(NB):
            q_s[b] = qkv[:, b * 128:(b + 1) * 128] * (DH ** -0.5)
            k_s[b, PAD:, :] = qkv[:, D + b * 128:D + (b + 1) * 128]
            v_s[b, PAD:, :] = qkv[:, 2 * D + b * 128:2 * D + (b + 1) * 128]
        for s0 in range(0, TA, 16):
            q = [q_s[b, s0:s0 + 16, :] for b in range(NB)]
            lg = []
            for w in range(W):
                o = PAD + s0 - DIL * w
                a = q[0] * k_s[0, o:o + 16, :]
                for b in range(1, NB):
                    a = a + q[b] * k_s[b, o:o + 16, :]
                a = a + pltpu.roll(a, 64, 1)
                a = a + pltpu.roll(a, 32, 1)
                if s0 < DIL * w:
                    pos = r0 + s0 + jax.lax.broadcasted_iota(
                        jnp.int32, (16, 128), 0)
                    a = jnp.where(pos >= DIL * w, a, -1e9)
                lg.append(a)
            m = lg[0]
            for w in range(1, W):
                m = jnp.maximum(m, lg[w])
            p = [jnp.exp(a - m) for a in lg]
            den = p[0]
            for w in range(1, W):
                den = den + p[w]
            inv = 1.0 / den
            p = [pw * inv for pw in p]
            for b in range(NB):
                acc = p[0] * v_s[b, PAD + s0:PAD + s0 + 16, :]
                for w in range(1, W):
                    o = PAD + s0 - DIL * w
                    acc = acc + p[w] * v_s[b, o:o + 16, :]
                o_s[s0:s0 + 16, b * 128:(b + 1) * 128] = acc.astype(bf16)
        k_s[:, :PAD, :] = k_s[:, TA:, :]
        v_s[:, :PAD, :] = v_s[:, TA:, :]
        xn = xs[pl.ds(r0, TA), :] + _dot(o_s[...], wo[...])
        xs[pl.ds(r0, TA), :] = xn
        xc, var = _ln_stats(xn)
        r = jax.lax.rsqrt(var + EPS)
        r = r * jax.lax.rsqrt(var * r * r + EPS)
        ht[:, pl.ds(r0, TA)] = (xc * r).astype(bf16).T
        return 0

    def mix1(j, _):
        c = pl.multiple_of(j * TF, TF)
        u = _dot(ht[...], w1[:, pl.ds(c, TF)]) + b1_ref[:, pl.ds(c, TF)].astype(f32)
        g_s[:, pl.ds(c, TF)] = jax.nn.gelu(u, approximate=True).astype(bf16)
        return 0

    def mix2(j, _):
        c = pl.multiple_of(j * TS, TS)
        y = _dot(g_s[...], w2[:, pl.ds(c, TS)]) + b2_ref[:, pl.ds(c, TS)].astype(f32)
        xs[pl.ds(c, TS), :] = xs[pl.ds(c, TS), :] + y.T
        return 0

    def layer(l, _):
        k_s[:, :PAD, :] = jnp.zeros((NB, PAD, 128), f32)
        v_s[:, :PAD, :] = jnp.zeros((NB, PAD, 128), f32)
        jax.lax.fori_loop(0, S // TA, attn_block, 0)

        @pl.when(l == 0)
        def _():
            cp_w1.wait()
        jax.lax.fori_loop(0, F // TF, mix1, 0)

        @pl.when(l == 0)
        def _():
            cp_w2.wait()
        jax.lax.fori_loop(0, S // TS, mix2, 0)
        return 0

    jax.lax.fori_loop(0, 2, layer, 0)
    xin[...] = xs[...].astype(bf16)
    cp_o = pltpu.make_async_copy(xin, out_hbm, sems.at[0])
    cp_o.start()
    cp_o.wait()


@jax.jit
def pallas_interleave_layers__sliding_local_dilated__mixer_token_mlp__prompt_kernel(
    A_x: jax.Array,
    A_wqkv: jax.Array,
    A_wo: jax.Array,
    B_x: jax.Array,
    B_w1: jax.Array,
    B_b1: jax.Array,
    B_w2: jax.Array,
    B_b2: jax.Array,
):
    del B_x
    hbm = pl.BlockSpec(memory_space=pl.ANY)
    vmem = pl.BlockSpec(memory_space=pltpu.VMEM)
    out = pl.pallas_call(
        _kernel,
        in_specs=[hbm, hbm, hbm, hbm, vmem, hbm, vmem],
        out_specs=hbm,
        out_shape=jax.ShapeDtypeStruct((S, D), bf16),
        scratch_shapes=[
            pltpu.VMEM((S, D), bf16),
            pltpu.VMEM((D, 3 * D), bf16),
            pltpu.VMEM((D, D), bf16),
            pltpu.VMEM((S, F), bf16),
            pltpu.VMEM((F, S), bf16),
            pltpu.VMEM((S, D), f32),
            pltpu.VMEM((D, 128), jnp.uint32),
            pltpu.VMEM((D, 128), f32),
            pltpu.VMEM((NB, TA, 128), f32),
            pltpu.VMEM((NB, PAD + TA, 128), f32),
            pltpu.VMEM((NB, PAD + TA, 128), f32),
            pltpu.VMEM((TA, D), bf16),
            pltpu.VMEM((D, S), bf16),
            pltpu.VMEM((D, F), bf16),
            pltpu.SemaphoreType.DMA((5,)),
        ],
        compiler_params=pltpu.CompilerParams(
            vmem_limit_bytes=110 * 1024 * 1024),
    )(A_x.reshape(S, D), A_wqkv, A_wo, B_w1, B_b1.reshape(1, F), B_w2,
      B_b2.reshape(1, S))
    return out.reshape(1, S, D)
```

```python
import jax
import jax.numpy as jnp
import numpy as np
import jax.experimental.pallas as pl
import jax.experimental.pallas.tpu as pltpu

S, D, F = 2048, 1024, 3584
H, DH, W, DIL = 32, 32, 8, 2
EPS = 1e-5
PAD = 16
TA = 256
TF = 512
TS = 512
NB = D // 128
NA = S // TA
f32, bf16 = jnp.float32, jnp.bfloat16


def _loop(name, n, body):
    with jax.named_scope(name):
        jax.lax.fori_loop(0, n, body, 0)


def _dot(a, b):
    return jnp.dot(a, b, preferred_element_type=f32)


def _ln_stats(x):
    m = jnp.mean(x, axis=-1, keepdims=True)
    xc = x - m
    v = jnp.mean(xc * xc, axis=-1, keepdims=True)
    return xc, v


def _head_minor_rows(tmp):
    return jnp.concatenate(
        [tmp[pl.ds(c, H, stride=DH), :] for c in range(DH)], axis=0)


def _kernel(x_hbm, wqkv_hbm, wo_hbm, w1_hbm, b1_ref, w2_hbm, b2_ref, out_hbm,
            xin, wqkv, wo, w1, w2, xs, tmpu, tmpf, ln_s, q_s, k_s, v_s, p_s,
            o_s, ht, g_s, b1_s, b2_s, sems, xsems):
    def rows(i, n):
        return pl.ds(i * n if isinstance(i, int) else pl.multiple_of(i * n, n), n)

    def cp_x(i):
        return pltpu.make_async_copy(
            x_hbm.at[rows(i, TA)], xin.at[rows(i, TA)], xsems.at[i])

    def cp_out(j):
        return pltpu.make_async_copy(
            xin.at[rows(j, TS)], out_hbm.at[rows(j, TS)], xsems.at[j])

    def cp_qkv(i):
        return pltpu.make_async_copy(
            wqkv_hbm.at[rows(i, 256)], wqkv.at[rows(i, 256)], sems.at[3 + i])

    cp_wo = pltpu.make_async_copy(wo_hbm, wo, sems.at[0])

    def cp_w1(j):
        c = rows(j, TF)
        return pltpu.make_async_copy(w1_hbm.at[:, c], w1.at[:, c], sems.at[1])

    def cp_w2(j):
        c = rows(j, TF)
        return pltpu.make_async_copy(w2_hbm.at[c], w2.at[c], sems.at[2])

    cp_qkv(0).start()
    cp_qkv(1).start()
    b1_s[...] = b1_ref[...].astype(f32).reshape(1, F)
    b2_s[...] = b2_ref[...].astype(f32).reshape(1, S)

    def perm_qkv(i, _):
        cp_qkv(i).wait()

        @pl.when(i == 0)
        def _():
            cp_qkv(2).start()
            cp_qkv(3).start()
            for j in range(3):
                cp_x(j).start()
            cp_wo.start()

        for t in range(3):
            c = slice(t * D, (t + 1) * D)
            tmpu[t] = pltpu.bitcast(wqkv[rows(i, 256), c], jnp.uint32).T
        for t in range(3):
            c = slice(t * D, (t + 1) * D)
            wqkv[rows(i, 256), c] = pltpu.bitcast(
                _head_minor_rows(tmpu.at[t]).T, bf16)
        return 0
    _loop("perm_qkv", 4, perm_qkv)

    cp_wo.wait()

    def perm_wo(i, _):
        for t in range(2):
            tmpf[t] = wo[:, rows(2 * i + t, 128)].astype(f32)
        for t in range(2):
            wo[:, rows(2 * i + t, 128)] = _head_minor_rows(tmpf.at[t]).astype(bf16)
        return 0

    def load_x(l, i):
        @pl.when(l == 0)
        def _():
            cp_x(i).wait()
            xs[rows(i, TA), :] = xin[rows(i, TA), :].astype(f32)

    TQ = TA

    def st_ln(i):
        xc, var = _ln_stats(xs[rows(i, TQ), :])
        ln_s[...] = (xc * jax.lax.rsqrt(var + EPS)).astype(bf16)

    def st_proj():
        k_s[:, :PAD, :] = k_s[:, TA:, :]
        v_s[:, :PAD, :] = v_s[:, TA:, :]
        qkv = _dot(ln_s[...], wqkv[...])
        for b in range(NB):
            q_s[b] = qkv[:, b * 128:(b + 1) * 128]
            k_s[b, PAD:, :] = qkv[:, D + b * 128:D + (b + 1) * 128]
            v_s[b, PAD:, :] = qkv[:, 2 * D + b * 128:2 * D + (b + 1) * 128]

    def st_logits(c, first):
        base = 0
        for s0 in range(0, TQ, 8):
            q = [q_s[b, pl.ds(base + s0, 8), :] for b in range(NB)]
            lg = []
            for w in range(W):
                o = base + (PAD + s0 - DIL * w)
                a = q[0] * k_s[0, pl.ds(o, 8), :]
                for b in range(1, NB):
                    a = a + q[b] * k_s[b, pl.ds(o, 8), :]
                a = a + pltpu.roll(a, 64, 1)
                a = (a + pltpu.roll(a, 32, 1)) * (DH ** -0.5)
                if first and s0 < DIL * w:
                    pos = base + s0 + jax.lax.broadcasted_iota(jnp.int32, (8, 128), 0)
                    a = jnp.where(pos >= DIL * w, a, -1e9)
                lg.append(a)
            m = lg[0]
            for w in range(1, W):
                m = jnp.maximum(m, lg[w])
            p = [jnp.exp(a - m) for a in lg]
            den = p[0]
            for w in range(1, W):
                den = den + p[w]
            inv = 1.0 / den
            for w in range(W):
                p_s[w, pl.ds(base + s0, 8), :] = p[w] * inv

    def st_pv(c):
        base = 0
        for s0 in range(0, TQ, 16):
            p = [p_s[w, pl.ds(base + s0, 16), :] for w in range(W)]
            for b in range(NB):
                acc = p[0] * v_s[b, pl.ds(base + PAD + s0, 16), :]
                for w in range(1, W):
                    o = base + (PAD + s0 - DIL * w)
                    acc = acc + p[w] * v_s[b, pl.ds(o, 16), :]
                o_s[pl.ds(s0, 16), b * 128:(b + 1) * 128] = acc.astype(bf16)

    def st_wo(i):
        c = slice(None)
        xs[rows(i, TA), c] = xs[rows(i, TA), c] + _dot(o_s[...], wo[:, c])

    def st_h(i, c):
        xc, var = _ln_stats(xs[rows(i, TQ), :])
        r = jax.lax.rsqrt(var + EPS)
        r = r * jax.lax.rsqrt(var * r * r + EPS)
        ht[:, rows(i, TA)] = (xc * r).astype(bf16).T

    def attn_step(i, first=False, last=False):
        if not first:
            st_pv(0)
        if not last:
            st_proj()
            st_logits(0, first)
            st_ln(jnp.minimum(i + 1, NA - 1))
        if not first:
            st_h(jnp.maximum(i - 2, 0), 0)
            st_wo(i - 1)

    def mix1(j, _):
        c = rows(j, TF)
        u = _dot(ht[...], w1[:, c]) + b1_s[:, c]
        g_s[:, c] = jax.nn.gelu(u, approximate=True).astype(bf16)
        return 0

    def layer(l, _):
        load_x(l, 0)
        load_x(l, 1)
        with jax.named_scope("pro"):
            st_ln(0)
            k_s[:, TA:, :] = jnp.zeros((NB, PAD, 128), f32)
            v_s[:, TA:, :] = jnp.zeros((NB, PAD, 128), f32)
            attn_step(0, first=True)
            if l == 0:
                for c in range(NB // 2):
                    perm_wo(c, 0)

        def attn_block(j, _):
            i = j + 1

            if l == 0:
                @pl.when(i + 1 < NA)
                def _():
                    @pl.when(i + 2 < NA)
                    def _():
                        cp_x(i + 2).start()
                    cp_w1(j).start()
                    load_x(l, i + 1)

                @pl.when(i + 1 == NA)
                def _():
                    cp_w1(j).start()
            attn_step(i)
            return 0
        _loop("attn_block", NA - 1, attn_block)
        with jax.named_scope("epi"):
            attn_step(NA, last=True)
            st_h(NA - 1, 0)

        @pl.when(l == 0)
        def _():
            for j in range(F // TF):
                cp_w1(j).wait()

        def mix1_(j, _):
            @pl.when(l == 0)
            def _():
                cp_w2(j).start()
            return mix1(j, 0)
        _loop("mix1", F // TF, mix1_)

        @pl.when(l == 0)
        def _():
            for j in range(F // TF):
                cp_w2(j).wait()

        def mix2(j, _):
            c = rows(j, TS)
            y = _dot(g_s[...], w2[:, c]) + b2_s[:, c]
            xn = xs[c, :] + y.T
            xs[c, :] = xn
            xin[c, :] = xn.astype(bf16)

            @pl.when(l == 1)
            def _():
                cp_out(j).start()
            return 0
        _loop("mix2", S // TS, mix2)
        return 0

    layer(0, 0)
    layer(1, 0)
    for j in range(S // TS):
        cp_out(j).wait()


@jax.jit
def pallas_interleave_layers__sliding_local_dilated__mixer_token_mlp__prompt_kernel(
    A_x: jax.Array,
    A_wqkv: jax.Array,
    A_wo: jax.Array,
    B_x: jax.Array,
    B_w1: jax.Array,
    B_b1: jax.Array,
    B_w2: jax.Array,
    B_b2: jax.Array,
):
    del B_x
    hbm = pl.BlockSpec(memory_space=pl.ANY)
    vmem = pl.BlockSpec(memory_space=pltpu.VMEM)
    out = pl.pallas_call(
        _kernel,
        in_specs=[hbm, hbm, hbm, hbm, vmem, hbm, vmem],
        out_specs=hbm,
        out_shape=jax.ShapeDtypeStruct((S, D), bf16),
        scratch_shapes=[
            pltpu.VMEM((S, D), bf16),
            pltpu.VMEM((D, 3 * D), bf16),
            pltpu.VMEM((D, D), bf16),
            pltpu.VMEM((S, F), bf16),
            pltpu.VMEM((F, S), bf16),
            pltpu.VMEM((S, D), f32),
            pltpu.VMEM((3, D, 128), jnp.uint32),
            pltpu.VMEM((2, D, 128), f32),
            pltpu.VMEM((TA, D), bf16),
            pltpu.VMEM((NB, TA, 128), f32),
            pltpu.VMEM((NB, PAD + TA, 128), f32),
            pltpu.VMEM((NB, PAD + TA, 128), f32),
            pltpu.VMEM((W, TA, 128), f32),
            pltpu.VMEM((TA, D), bf16),
            pltpu.VMEM((D, S), bf16),
            pltpu.VMEM((D, F), bf16),
            pltpu.VMEM((1, F), f32),
            pltpu.VMEM((1, S), f32),
            pltpu.SemaphoreType.DMA((7,)),
            pltpu.SemaphoreType.DMA((max(NA, S // TS),)),
        ],
        compiler_params=pltpu.CompilerParams(
            vmem_limit_bytes=110 * 1024 * 1024),
    )(A_x.reshape(S, D), A_wqkv, A_wo, B_w1, B_b1, B_w2,
      B_b2)
    return out.reshape(1, S, D)
```

```python
import jax
import jax.numpy as jnp
import numpy as np
import jax.experimental.pallas as pl
import jax.experimental.pallas.tpu as pltpu

S, D, F = 2048, 1024, 3584
H, DH, W, DIL = 32, 32, 8, 2
EPS = 1e-5
PAD = 16
TA = 256
TF = 512
TS = 512
NB = D // 128
NA = S // TA
f32, bf16 = jnp.float32, jnp.bfloat16


def _loop(name, n, body):
    with jax.named_scope(name):
        jax.lax.fori_loop(0, n, body, 0)


def _dot(a, b):
    return jnp.dot(a, b, preferred_element_type=f32)


def _ln_stats(x):
    m = jnp.mean(x, axis=-1, keepdims=True)
    xc = x - m
    v = jnp.mean(xc * xc, axis=-1, keepdims=True)
    return xc, v


def _put_rows(tmp, val):
    for h in range(H):
        tmp[h * (DH + 1):h * (DH + 1) + DH, :] = val[h * DH:(h + 1) * DH]


def _head_minor_rows(tmp):
    return jnp.concatenate(
        [tmp[pl.ds(c, H, stride=DH + 1), :] for c in range(DH)], axis=0)


def _kernel(x_hbm, wqkv_hbm, wo_hbm, w1_hbm, b1_ref, w2_hbm, b2_ref, out_hbm,
            xin, wqkv, wo, w1, w2, xs, tmpu, tmpf, ln_s, q_s, k_s, v_s, p_s,
            o_s, ht, g_s, b1_s, b2_s, sems, xsems):
    def rows(i, n):
        return pl.ds(i * n if isinstance(i, int) else pl.multiple_of(i * n, n), n)

    def cp_x(i):
        return pltpu.make_async_copy(
            x_hbm.at[rows(i, TA)], xin.at[rows(i, TA)], xsems.at[i])

    def cp_out(j):
        return pltpu.make_async_copy(
            xin.at[rows(j, TS)], out_hbm.at[rows(j, TS)], xsems.at[j])

    def cp_qkv(i):
        return pltpu.make_async_copy(
            wqkv_hbm.at[rows(i, 256)], wqkv.at[rows(i, 256)], sems.at[3 + i])

    cp_wo = pltpu.make_async_copy(wo_hbm, wo, sems.at[0])

    def cp_w1(j):
        c = rows(j, TF)
        return pltpu.make_async_copy(w1_hbm.at[:, c], w1.at[:, c], sems.at[1])

    def cp_w2(j):
        c = rows(j, TF)
        return pltpu.make_async_copy(w2_hbm.at[c], w2.at[c], sems.at[2])

    cp_qkv(0).start()
    cp_qkv(1).start()
    b1_s[...] = b1_ref[...].astype(f32).reshape(1, F)
    b2_s[...] = b2_ref[...].astype(f32).reshape(1, S)

    def perm_qkv(i, _):
        cp_qkv(i).wait()

        @pl.when(i < 2)
        def _():
            cp_qkv(i + 2).start()

        @pl.when(i >= 2)
        def _():
            cp_x(i - 2).start()

        for t in range(3):
            c = slice(t * D, (t + 1) * D)
            _put_rows(tmpu.at[t],
                      pltpu.bitcast(wqkv[rows(i, 256), c], jnp.uint32).T)
        for t in range(3):
            c = slice(t * D, (t + 1) * D)
            wqkv[rows(i, 256), c] = pltpu.bitcast(
                _head_minor_rows(tmpu.at[t]).T, bf16)
        return 0
    _loop("perm_qkv", 4, perm_qkv)

    def perm_wo(i, _):
        for t in range(2):
            _put_rows(tmpf.at[t], wo[:, rows(2 * i + t, 128)].astype(f32))
        for t in range(2):
            wo[:, rows(2 * i + t, 128)] = _head_minor_rows(tmpf.at[t]).astype(bf16)
        return 0

    def load_x(l, i):
        @pl.when(l == 0)
        def _():
            cp_x(i).wait()
            xs[rows(i, TA), :] = xin[rows(i, TA), :].astype(f32)

    TQ = TA

    def st_ln(i):
        xc, var = _ln_stats(xs[rows(i, TQ), :])
        ln_s[...] = (xc * jax.lax.rsqrt(var + EPS)).astype(bf16)

    def st_proj():
        k_s[:, :PAD, :] = k_s[:, TA:, :]
        v_s[:, :PAD, :] = v_s[:, TA:, :]
        qkv = _dot(ln_s[...], wqkv[...])
        for b in range(NB):
            q_s[b] = qkv[:, b * 128:(b + 1) * 128]
            k_s[b, PAD:, :] = qkv[:, D + b * 128:D + (b + 1) * 128]
            v_s[b, PAD:, :] = qkv[:, 2 * D + b * 128:2 * D + (b + 1) * 128]

    def st_logits(c, first):
        base = 0
        for s0 in range(0, TQ, 8):
            q = [q_s[b, pl.ds(base + s0, 8), :] for b in range(NB)]
            lg = []
            for w in range(W):
                o = base + (PAD + s0 - DIL * w)
                a = q[0] * k_s[0, pl.ds(o, 8), :]
                for b in range(1, NB):
                    a = a + q[b] * k_s[b, pl.ds(o, 8), :]
                a = a + pltpu.roll(a, 64, 1)
                a = (a + pltpu.roll(a, 32, 1)) * (DH ** -0.5)
                if first and s0 < DIL * w:
                    pos = base + s0 + jax.lax.broadcasted_iota(jnp.int32, (8, 128), 0)
                    a = jnp.where(pos >= DIL * w, a, -1e9)
                lg.append(a)
            m = lg[0]
            for w in range(1, W):
                m = jnp.maximum(m, lg[w])
            p = [jnp.exp(a - m) for a in lg]
            den = p[0]
            for w in range(1, W):
                den = den + p[w]
            inv = 1.0 / den
            for w in range(W):
                p_s[w, pl.ds(base + s0, 8), :] = p[w] * inv

    def st_pv(c):
        base = 0
        for s0 in range(0, TQ, 16):
            p = [p_s[w, pl.ds(base + s0, 16), :] for w in range(W)]
            for b in range(NB):
                acc = p[0] * v_s[b, pl.ds(base + PAD + s0, 16), :]
                for w in range(1, W):
                    o = base + (PAD + s0 - DIL * w)
                    acc = acc + p[w] * v_s[b, pl.ds(o, 16), :]
                o_s[pl.ds(s0, 16), b * 128:(b + 1) * 128] = acc.astype(bf16)

    def st_wo(i):
        c = slice(None)
        xs[rows(i, TA), c] = xs[rows(i, TA), c] + _dot(o_s[...], wo[:, c])

    def st_h(i, c):
        xc, var = _ln_stats(xs[rows(i, TQ), :])
        r = jax.lax.rsqrt(var + EPS)
        r = r * jax.lax.rsqrt(var * r * r + EPS)
        ht[:, rows(i, TA)] = (xc * r).astype(bf16).T

    def attn_step(i, first=False, last=False):
        if not first:
            st_pv(0)
        if not last:
            st_proj()
            st_logits(0, first)
            st_ln(jnp.minimum(i + 1, NA - 1))
        if not first:
            st_h(jnp.maximum(i - 2, 0), 0)
            st_wo(i - 1)

    def mix1(j, _):
        c = rows(j, TF)
        u = _dot(ht[...], w1[:, c]) + b1_s[:, c]
        g_s[:, c] = jax.nn.gelu(u, approximate=True).astype(bf16)
        return 0

    def layer(l, _):
        load_x(l, 0)
        load_x(l, 1)
        if l == 0:
            cp_wo.start()
            cp_x(2).start()
        with jax.named_scope("pro"):
            st_ln(0)
            k_s[:, TA:, :] = jnp.zeros((NB, PAD, 128), f32)
            v_s[:, TA:, :] = jnp.zeros((NB, PAD, 128), f32)
            attn_step(0, first=True)
            if l == 0:
                cp_wo.wait()
                jax.lax.fori_loop(0, NB // 2, perm_wo, 0)

        def attn_block(j, _):
            i = j + 1

            if l == 0:
                @pl.when(i + 1 < NA)
                def _():
                    @pl.when(i + 2 < NA)
                    def _():
                        cp_x(i + 2).start()
                    cp_w1(j).start()
                    load_x(l, i + 1)

                @pl.when(i + 1 == NA)
                def _():
                    cp_w1(j).start()
            attn_step(i)
            return 0
        _loop("attn_block", NA - 1, attn_block)
        with jax.named_scope("epi"):
            attn_step(NA, last=True)
            st_h(NA - 1, 0)

        @pl.when(l == 0)
        def _():
            for j in range(F // TF):
                cp_w1(j).wait()

        def mix1_(j, _):
            @pl.when(l == 0)
            def _():
                cp_w2(j).start()
            return mix1(j, 0)
        _loop("mix1", F // TF, mix1_)

        @pl.when(l == 0)
        def _():
            for j in range(F // TF):
                cp_w2(j).wait()

        def mix2(j, _):
            c = rows(j, TS)
            y = _dot(g_s[...], w2[:, c]) + b2_s[:, c]
            xn = xs[c, :] + y.T
            xs[c, :] = xn
            xin[c, :] = xn.astype(bf16)

            @pl.when(l == 1)
            def _():
                cp_out(j).start()
            return 0
        _loop("mix2", S // TS, mix2)
        return 0

    layer(0, 0)
    layer(1, 0)
    for j in range(S // TS):
        cp_out(j).wait()


@jax.jit
def pallas_interleave_layers__sliding_local_dilated__mixer_token_mlp__prompt_kernel(
    A_x: jax.Array,
    A_wqkv: jax.Array,
    A_wo: jax.Array,
    B_x: jax.Array,
    B_w1: jax.Array,
    B_b1: jax.Array,
    B_w2: jax.Array,
    B_b2: jax.Array,
):
    del B_x
    hbm = pl.BlockSpec(memory_space=pl.ANY)
    vmem = pl.BlockSpec(memory_space=pltpu.VMEM)
    out = pl.pallas_call(
        _kernel,
        in_specs=[hbm, hbm, hbm, hbm, vmem, hbm, vmem],
        out_specs=hbm,
        out_shape=jax.ShapeDtypeStruct((S, D), bf16),
        scratch_shapes=[
            pltpu.VMEM((S, D), bf16),
            pltpu.VMEM((D, 3 * D), bf16),
            pltpu.VMEM((D, D), bf16),
            pltpu.VMEM((S, F), bf16),
            pltpu.VMEM((F, S), bf16),
            pltpu.VMEM((S, D), f32),
            pltpu.VMEM((3, D + H, 128), jnp.uint32),
            pltpu.VMEM((2, D + H, 128), f32),
            pltpu.VMEM((TA, D), bf16),
            pltpu.VMEM((NB, TA, 128), f32),
            pltpu.VMEM((NB, PAD + TA, 128), f32),
            pltpu.VMEM((NB, PAD + TA, 128), f32),
            pltpu.VMEM((W, TA, 128), f32),
            pltpu.VMEM((TA, D), bf16),
            pltpu.VMEM((D, S), bf16),
            pltpu.VMEM((D, F), bf16),
            pltpu.VMEM((1, F), f32),
            pltpu.VMEM((1, S), f32),
            pltpu.SemaphoreType.DMA((7,)),
            pltpu.SemaphoreType.DMA((max(NA, S // TS),)),
        ],
        compiler_params=pltpu.CompilerParams(
            vmem_limit_bytes=110 * 1024 * 1024),
    )(A_x.reshape(S, D), A_wqkv, A_wo, B_w1, B_b1, B_w2,
      B_b2)
    return out.reshape(1, S, D)
```

```python
import jax
import jax.numpy as jnp
import numpy as np
import jax.experimental.pallas as pl
import jax.experimental.pallas.tpu as pltpu

S, D, F = 2048, 1024, 3584
H, DH, W, DIL = 32, 32, 8, 2
EPS = 1e-5
PAD = 16
TA = 256
TF = 512
TS = 512
NB = D // 128
HD = D // 2
NA = S // TA
f32, bf16 = jnp.float32, jnp.bfloat16


def _loop(name, n, body):
    with jax.named_scope(name):
        jax.lax.fori_loop(0, n, body, 0)


def _dot(a, b):
    return jnp.dot(a, b, preferred_element_type=f32)


def _ln_stats(x):
    m = jnp.mean(x, axis=-1, keepdims=True)
    xc = x - m
    v = jnp.mean(xc * xc, axis=-1, keepdims=True)
    return xc, v


def _words(v):
    return pltpu.bitcast(v, jnp.uint32)


def _strassen_lhs(a11, a12, a21, a22):
    return [a11 + a22, a21 + a22, a11, a22, a11 + a12, a21 - a11, a12 - a22]


def _strassen_rhs(b11, b12, b21, b22):
    return [b11 + b22, b11, b12 - b22, b21 - b11, b22, b11 + b12, b21 + b22]


def _strassen(lhs, rhs, c):
    m1, m2, m3, m4, m5, m6, m7 = [
        _dot(pltpu.bitcast(lhs[n], bf16), pltpu.bitcast(rhs[n, :, c], bf16))
        for n in range(7)]
    return m1 + m4 - m5 + m7, m3 + m5, m2 + m4, m1 - m2 + m3 + m6


def _put_rows(tmp, val):
    for h in range(H):
        tmp[h * (DH + 1):h * (DH + 1) + DH, :] = val[h * DH:(h + 1) * DH]


def _head_minor_rows(tmp):
    return jnp.concatenate(
        [tmp[pl.ds(c, H, stride=DH + 1), :] for c in range(DH)], axis=0)


def _kernel(x_hbm, wqkv_hbm, wo_hbm, w1_hbm, b1_ref, w2_hbm, b2_ref, out_hbm,
            xin, wqkv, wo, w1, w2, w1c, w2c, xs, tmpu, tmpf, ln_s, q_s, k_s, v_s, p_s,
            o_s, ht, g_s, b1_s, b2_s, sems, xsems):
    def rows(i, n):
        return pl.ds(i * n if isinstance(i, int) else pl.multiple_of(i * n, n), n)

    def cp_x(i):
        return pltpu.make_async_copy(
            x_hbm.at[rows(i, TA)], xin.at[rows(i, TA)], xsems.at[i])

    def cp_out(j):
        return pltpu.make_async_copy(
            xin.at[rows(j, TS)], out_hbm.at[rows(j, TS)], xsems.at[j])

    def cp_qkv(i):
        return pltpu.make_async_copy(
            wqkv_hbm.at[rows(i, 256)], wqkv.at[rows(i, 256)], sems.at[3 + i])

    cp_wo = pltpu.make_async_copy(wo_hbm, wo, sems.at[0])

    def cp_w1(j):
        c = rows(j, TF)
        return pltpu.make_async_copy(w1_hbm.at[:, c], w1.at[j % 3],
                                     sems.at[7 + j % 3])

    def cp_w2(j):
        c = rows(j, TF)
        return pltpu.make_async_copy(w2_hbm.at[c], w2.at[j % 3], sems.at[10 + j % 3])

    cp_qkv(0).start()
    cp_qkv(1).start()
    b1_s[...] = b1_ref[...].astype(f32).reshape(1, F)
    b2_s[...] = b2_ref[...].astype(f32).reshape(1, S)

    def perm_qkv(i, _):
        cp_qkv(i).wait()

        @pl.when(i < 2)
        def _():
            cp_qkv(i + 2).start()

        @pl.when(i >= 2)
        def _():
            cp_x(i - 2).start()

        for t in range(3):
            c = slice(t * D, (t + 1) * D)
            _put_rows(tmpu.at[t],
                      pltpu.bitcast(wqkv[rows(i, 256), c], jnp.uint32).T)
        for t in range(3):
            c = slice(t * D, (t + 1) * D)
            wqkv[rows(i, 256), c] = pltpu.bitcast(
                _head_minor_rows(tmpu.at[t]).T, bf16)
        return 0
    _loop("perm_qkv", 4, perm_qkv)

    def perm_wo(i, _):
        for t in range(2):
            _put_rows(tmpf.at[t], wo[:, rows(2 * i + t, 128)].astype(f32))
        for t in range(2):
            wo[:, rows(2 * i + t, 128)] = _head_minor_rows(tmpf.at[t]).astype(bf16)
        return 0

    def load_x(l, i):
        @pl.when(l == 0)
        def _():
            cp_x(i).wait()
            xs[rows(i, TA), :] = xin[rows(i, TA), :].astype(f32)

    TQ = TA

    def st_ln(i):
        xc, var = _ln_stats(xs[rows(i, TQ), :])
        ln_s[...] = (xc * jax.lax.rsqrt(var + EPS)).astype(bf16)

    def st_proj():
        k_s[:, :PAD, :] = k_s[:, TA:, :]
        v_s[:, :PAD, :] = v_s[:, TA:, :]
        qkv = _dot(ln_s[...], wqkv[...])
        for b in range(NB):
            q_s[b] = qkv[:, b * 128:(b + 1) * 128]
            k_s[b, PAD:, :] = qkv[:, D + b * 128:D + (b + 1) * 128]
            v_s[b, PAD:, :] = qkv[:, 2 * D + b * 128:2 * D + (b + 1) * 128]

    def st_logits(c, first):
        base = 0
        for s0 in range(0, TQ, 8):
            q = [q_s[b, pl.ds(base + s0, 8), :] for b in range(NB)]
            lg = []
            for w in range(W):
                o = base + (PAD + s0 - DIL * w)
                a = q[0] * k_s[0, pl.ds(o, 8), :]
                for b in range(1, NB):
                    a = a + q[b] * k_s[b, pl.ds(o, 8), :]
                a = a + pltpu.roll(a, 64, 1)
                a = (a + pltpu.roll(a, 32, 1)) * (DH ** -0.5)
                if first and s0 < DIL * w:
                    pos = base + s0 + jax.lax.broadcasted_iota(jnp.int32, (8, 128), 0)
                    a = jnp.where(pos >= DIL * w, a, -1e9)
                lg.append(a)
            m = lg[0]
            for w in range(1, W):
                m = jnp.maximum(m, lg[w])
            p = [jnp.exp(a - m) for a in lg]
            den = p[0]
            for w in range(1, W):
                den = den + p[w]
            inv = 1.0 / den
            for w in range(W):
                p_s[w, pl.ds(base + s0, 8), :] = p[w] * inv

    def st_pv(c):
        base = 0
        for s0 in range(0, TQ, 16):
            p = [p_s[w, pl.ds(base + s0, 16), :] for w in range(W)]
            for b in range(NB):
                acc = p[0] * v_s[b, pl.ds(base + PAD + s0, 16), :]
                for w in range(1, W):
                    o = base + (PAD + s0 - DIL * w)
                    acc = acc + p[w] * v_s[b, pl.ds(o, 16), :]
                o_s[pl.ds(s0, 16), b * 128:(b + 1) * 128] = acc.astype(bf16)

    def st_wo(i):
        c = slice(None)
        xs[rows(i, TA), c] = xs[rows(i, TA), c] + _dot(o_s[...], wo[:, c])

    def st_h(i, c):
        xc, var = _ln_stats(xs[rows(i, TQ), :])
        r = jax.lax.rsqrt(var + EPS)
        r = r * jax.lax.rsqrt(var * r * r + EPS)
        h = xc * r
        for n, a in enumerate(_strassen_lhs(
                h[:128, :HD], h[128:, :HD], h[:128, HD:], h[128:, HD:])):
            ht[n, :, rows(i, 128)] = _words(a.astype(bf16).T)

    def prep(src, r, dr, c):
        b = [src[r + y:r + y + 16, c + x:c + x + 128].astype(f32)
             for y in (0, dr) for x in (0, 256)]
        return enumerate(_words(v.astype(bf16)) for v in _strassen_rhs(*b))

    def prep_w1(j):
        for t in range(NA):
            for r in range(0, 128, 16):
                for c in range(2):
                    for n, v in prep(w1.at[j % 3], t * TA + r, 128, c * 128):
                        w1c[n, pl.ds(t * 64 + r // 2, 8), rows(2 * j + c, 128)] = v

    def prep_w2(j):
        for t in range(S // TS):
            for r in range(16):
                for c in range(2):
                    for n, v in prep(w2.at[j % 3], r * 16, 256, t * TS + c * 128):
                        w2c[n, rows(j * 16 + r, 8), rows(2 * t + c, 128)] = v

    def stream(cp, j):
        cp(j).wait()

        @pl.when(j + 2 < F // TF)
        def _():
            cp(j + 2).start()

    def attn_step(i, first=False, last=False):
        if not first:
            st_pv(0)
        if not last:
            st_proj()
            st_logits(0, first)
            st_ln(jnp.minimum(i + 1, NA - 1))
        if not first:
            st_h(jnp.maximum(i - 2, 0), 0)
            st_wo(i - 1)

    def mix1(j, _):
        c = rows(j, TF)
        bias = b1_s[:, c]
        g = [jax.nn.gelu(u + bias[:, (n % 2) * 256:(n % 2 + 1) * 256],
                         approximate=True)
             for n, u in enumerate(_strassen(ht, w1c, rows(j, 256)))]
        for n, a in enumerate(_strassen_lhs(*g)):
            g_s[n, :, rows(j, 256)] = _words(a.astype(bf16))
        return 0

    def layer(l, _):
        load_x(l, 0)
        load_x(l, 1)
        if l == 0:
            cp_wo.start()
            cp_x(2).start()
            cp_w1(0).start()
            cp_w1(1).start()
        with jax.named_scope("pro"):
            st_ln(0)
            k_s[:, TA:, :] = jnp.zeros((NB, PAD, 128), f32)
            v_s[:, TA:, :] = jnp.zeros((NB, PAD, 128), f32)
            attn_step(0, first=True)
            if l == 0:
                cp_wo.wait()
                jax.lax.fori_loop(0, NB // 2, perm_wo, 0)

        def attn_block(j, _):
            i = j + 1

            if l == 0:
                @pl.when(i + 1 < NA)
                def _():
                    @pl.when(i + 2 < NA)
                    def _():
                        cp_x(i + 2).start()
                    load_x(l, i + 1)
                stream(cp_w1, j)
                prep_w1(j)
            attn_step(i)
            return 0
        _loop("attn_block", NA - 1, attn_block)
        if l == 0:
            cp_w2(0).start()
            cp_w2(1).start()
        with jax.named_scope("epi"):
            attn_step(NA, last=True)
            st_h(NA - 1, 0)

        def mix1_(j, _):
            if l == 0:
                stream(cp_w2, j)
                prep_w2(j)
            return mix1(j, 0)
        _loop("mix1", F // TF, mix1_)

        def mix2(j, _):
            bias = b2_s[:, rows(j, TS)]
            for n, y in enumerate(_strassen(g_s, w2c, rows(j, 256))):
                y = y + bias[:, (n % 2) * 256:(n % 2 + 1) * 256]
                at = (rows(2 * j + n % 2, 256), rows(n // 2, HD))
                xn = xs[at] + y.T
                if l == 0:
                    xs[at] = xn
                else:
                    xin[at] = xn.astype(bf16)

            @pl.when(l == 1)
            def _():
                cp_out(j).start()
            return 0
        _loop("mix2", S // TS, mix2)
        return 0

    layer(0, 0)
    layer(1, 0)
    for j in range(S // TS):
        cp_out(j).wait()


@jax.jit
def pallas_interleave_layers__sliding_local_dilated__mixer_token_mlp__prompt_kernel(
    A_x: jax.Array,
    A_wqkv: jax.Array,
    A_wo: jax.Array,
    B_x: jax.Array,
    B_w1: jax.Array,
    B_b1: jax.Array,
    B_w2: jax.Array,
    B_b2: jax.Array,
):
    del B_x
    hbm = pl.BlockSpec(memory_space=pl.ANY)
    vmem = pl.BlockSpec(memory_space=pltpu.VMEM)
    out = pl.pallas_call(
        _kernel,
        in_specs=[hbm, hbm, hbm, hbm, vmem, hbm, vmem],
        out_specs=hbm,
        out_shape=jax.ShapeDtypeStruct((S, D), bf16),
        scratch_shapes=[
            pltpu.VMEM((S, D), bf16),
            pltpu.VMEM((D, 3 * D), bf16),
            pltpu.VMEM((D, D), bf16),
            pltpu.VMEM((3, S, TF), bf16),
            pltpu.VMEM((3, TF, S), bf16),
            pltpu.VMEM((7, S // 4, F // 2), jnp.uint32),
            pltpu.VMEM((7, F // 4, S // 2), jnp.uint32),
            pltpu.VMEM((S, D), f32),
            pltpu.VMEM((3, D + H, 128), jnp.uint32),
            pltpu.VMEM((2, D + H, 128), f32),
            pltpu.VMEM((TA, D), bf16),
            pltpu.VMEM((NB, TA, 128), f32),
            pltpu.VMEM((NB, PAD + TA, 128), f32),
            pltpu.VMEM((NB, PAD + TA, 128), f32),
            pltpu.VMEM((W, TA, 128), f32),
            pltpu.VMEM((TA, D), bf16),
            pltpu.VMEM((7, HD // 2, S // 2), jnp.uint32),
            pltpu.VMEM((7, HD // 2, F // 2), jnp.uint32),
            pltpu.VMEM((1, F), f32),
            pltpu.VMEM((1, S), f32),
            pltpu.SemaphoreType.DMA((13,)),
            pltpu.SemaphoreType.DMA((max(NA, S // TS),)),
        ],
        compiler_params=pltpu.CompilerParams(
            vmem_limit_bytes=124 * 1024 * 1024),
    )(A_x.reshape(S, D), A_wqkv, A_wo, B_w1, B_b1, B_w2,
      B_b2)
    return out.reshape(1, S, D)
```

```python
import jax
import jax.numpy as jnp
import numpy as np
import jax.experimental.pallas as pl
import jax.experimental.pallas.tpu as pltpu

S, D, F = 2048, 1024, 3584
H, DH, W, DIL = 32, 32, 8, 2
EPS = 1e-5
PAD = 16
TA = 256
TF = 512
TS = 512
NB = D // 128
HD = D // 2
NA = S // TA
f32, bf16 = jnp.float32, jnp.bfloat16


def _loop(name, n, body):
    with jax.named_scope(name):
        jax.lax.fori_loop(0, n, body, 0)


def _dot(a, b):
    return jnp.dot(a, b, preferred_element_type=f32)


def _ln_stats(x):
    m = jnp.mean(x, axis=-1, keepdims=True)
    xc = x - m
    v = jnp.mean(xc * xc, axis=-1, keepdims=True)
    return xc, v


def _words(v):
    return pltpu.bitcast(v, jnp.uint32)


def _strassen_lhs(a11, a12, a21, a22):
    return [a11 + a22, a21 + a22, a11, a22, a11 + a12, a21 - a11, a12 - a22]


def _strassen_rhs(b11, b12, b21, b22):
    return [b11 + b22, b11, b12 - b22, b21 - b11, b22, b11 + b12, b21 + b22]


def _strassen(lhs, rhs, c):
    m1, m2, m3, m4, m5, m6, m7 = [
        _dot(pltpu.bitcast(lhs[n], bf16), pltpu.bitcast(rhs[n, :, c], bf16))
        for n in range(7)]
    return m1 + m4 - m5 + m7, m3 + m5, m2 + m4, m1 - m2 + m3 + m6


def _put_rows(tmp, val):
    for h in range(H):
        tmp[h * (DH + 1):h * (DH + 1) + DH, :] = val[h * DH:(h + 1) * DH]


def _head_minor_rows(tmp):
    return jnp.concatenate(
        [tmp[pl.ds(c, H, stride=DH + 1), :] for c in range(DH)], axis=0)


def _kernel(x_hbm, wqkv_hbm, wo_hbm, w1_hbm, b1_ref, w2_hbm, b2_ref, out_hbm,
            xin, wqkv, wo, w1, w2, w1c, w2c, xs, tmpu, tmpf, ln_s, q_s, k_s, v_s, p_s,
            o_s, ht, g_s, b1_s, b2_s, sems, xsems):
    def rows(i, n):
        return pl.ds(i * n if isinstance(i, int) else pl.multiple_of(i * n, n), n)

    def cp_x(i):
        return pltpu.make_async_copy(
            x_hbm.at[rows(i, TA)], xin.at[rows(i, TA)], xsems.at[i])

    def cp_out(j):
        return pltpu.make_async_copy(
            xin.at[rows(j, TS)], out_hbm.at[rows(j, TS)], xsems.at[j])

    def cp_qkv(i):
        return pltpu.make_async_copy(
            wqkv_hbm.at[rows(i, 256)], wqkv.at[rows(i, 256)], sems.at[3 + i])

    cp_wo = pltpu.make_async_copy(wo_hbm, wo, sems.at[0])

    def cp_w1(j):
        c = rows(j, TF)
        return pltpu.make_async_copy(w1_hbm.at[:, c], w1.at[j % 3],
                                     sems.at[7 + j % 3])

    def cp_w2(j):
        c = rows(j, TF)
        return pltpu.make_async_copy(w2_hbm.at[c], w2.at[j % 3], sems.at[10 + j % 3])

    cp_qkv(0).start()
    cp_qkv(1).start()
    b1_s[...] = b1_ref[...].astype(f32).reshape(1, F)
    b2_s[...] = b2_ref[...].astype(f32).reshape(1, S)

    def perm_qkv(i, _):
        cp_qkv(i).wait()

        @pl.when(i < 2)
        def _():
            cp_qkv(i + 2).start()

        @pl.when(i >= 2)
        def _():
            cp_x(i - 2).start()

        for t in range(3):
            c = slice(t * D, (t + 1) * D)
            _put_rows(tmpu.at[t],
                      pltpu.bitcast(wqkv[rows(i, 256), c], jnp.uint32).T)
        for t in range(3):
            c = slice(t * D, (t + 1) * D)
            wqkv[rows(i, 256), c] = pltpu.bitcast(
                _head_minor_rows(tmpu.at[t]).T, bf16)
        return 0
    _loop("perm_qkv", 4, perm_qkv)

    def perm_wo(i, _):
        for t in range(2):
            _put_rows(tmpf.at[t], wo[:, rows(2 * i + t, 128)].astype(f32))
        for t in range(2):
            wo[:, rows(2 * i + t, 128)] = _head_minor_rows(tmpf.at[t]).astype(bf16)
        return 0

    def load_x(l, i):
        @pl.when(l == 0)
        def _():
            cp_x(i).wait()
            xs[rows(i, TA), :] = xin[rows(i, TA), :].astype(f32)

    TQ = TA

    def st_ln(i):
        xc, var = _ln_stats(xs[rows(i, TQ), :])
        ln_s[...] = (xc * jax.lax.rsqrt(var + EPS)).astype(bf16)

    def st_proj():
        k_s[:, :PAD, :] = k_s[:, TA:, :]
        v_s[:, :PAD, :] = v_s[:, TA:, :]
        qkv = _dot(ln_s[...], wqkv[...])
        for b in range(NB):
            q_s[b] = qkv[:, b * 128:(b + 1) * 128]
            k_s[b, PAD:, :] = qkv[:, D + b * 128:D + (b + 1) * 128]
            v_s[b, PAD:, :] = qkv[:, 2 * D + b * 128:2 * D + (b + 1) * 128]

    def st_logits(c, first):
        base = 0
        for s0 in range(0, TQ, 8):
            q = [q_s[b, pl.ds(base + s0, 8), :] for b in range(NB)]
            lg = []
            for w in range(W):
                o = base + (PAD + s0 - DIL * w)
                a = q[0] * k_s[0, pl.ds(o, 8), :]
                for b in range(1, NB):
                    a = a + q[b] * k_s[b, pl.ds(o, 8), :]
                a = a + pltpu.roll(a, 64, 1)
                a = (a + pltpu.roll(a, 32, 1)) * (DH ** -0.5)
                if first and s0 < DIL * w:
                    pos = base + s0 + jax.lax.broadcasted_iota(jnp.int32, (8, 128), 0)
                    a = jnp.where(pos >= DIL * w, a, -1e9)
                lg.append(a)
            m = lg[0]
            for w in range(1, W):
                m = jnp.maximum(m, lg[w])
            p = [jnp.exp(a - m) for a in lg]
            den = p[0]
            for w in range(1, W):
                den = den + p[w]
            inv = 1.0 / den
            for w in range(W):
                p_s[w, pl.ds(base + s0, 8), :] = p[w] * inv

    def st_pv(c):
        base = 0
        for s0 in range(0, TQ, 16):
            p = [p_s[w, pl.ds(base + s0, 16), :] for w in range(W)]
            for b in range(NB):
                acc = p[0] * v_s[b, pl.ds(base + PAD + s0, 16), :]
                for w in range(1, W):
                    o = base + (PAD + s0 - DIL * w)
                    acc = acc + p[w] * v_s[b, pl.ds(o, 16), :]
                o_s[pl.ds(s0, 16), b * 128:(b + 1) * 128] = acc.astype(bf16)

    def st_wo(i):
        c = slice(None)
        xs[rows(i, TA), c] = xs[rows(i, TA), c] + _dot(o_s[...], wo[:, c])

    def st_h(i, c):
        xc, var = _ln_stats(xs[rows(i, TQ), :])
        r = jax.lax.rsqrt(var + EPS)
        r = r * jax.lax.rsqrt(var * r * r + EPS)
        h = xc * r
        for n, a in enumerate(_strassen_lhs(
                h[:128, :HD], h[128:, :HD], h[:128, HD:], h[128:, HD:])):
            ht[n, :, rows(i, 128)] = _words(a.astype(bf16).T)

    def prep(src, r, dr, c):
        b = [_words(src[r + y:r + y + 16, c + x:c + x + 128])
             for y in (0, dr) for x in (0, 256)]
        lo = _strassen_rhs(*[pltpu.bitcast(v << 16, f32) for v in b])
        hi = _strassen_rhs(*[
            pltpu.bitcast(v & np.uint32(0xFFFF0000), f32) for v in b])
        out = [pltpu.pack_elementwise([x, y], packed_dtype=bf16)
               for x, y in zip(lo, hi)]
        out[1], out[4] = b[0], b[3]
        return enumerate(out)

    def prep_w1(j):
        for t in range(NA):
            for r in range(0, 128, 16):
                for c in range(2):
                    for n, v in prep(w1.at[j % 3], t * TA + r, 128, c * 128):
                        w1c[n, pl.ds(t * 64 + r // 2, 8), rows(2 * j + c, 128)] = v

    def prep_w2(j):
        for t in range(S // TS):
            for r in range(16):
                for c in range(2):
                    for n, v in prep(w2.at[j % 3], r * 16, 256, t * TS + c * 128):
                        w2c[n, rows(j * 16 + r, 8), rows(2 * t + c, 128)] = v

    def stream(cp, j):
        cp(j).wait()

        @pl.when(j + 2 < F // TF)
        def _():
            cp(j + 2).start()

    def attn_step(i, first=False, last=False):
        if not first:
            st_pv(0)
        if not last:
            st_proj()
            st_logits(0, first)
            st_ln(jnp.minimum(i + 1, NA - 1))
        if not first:
            st_h(jnp.maximum(i - 2, 0), 0)
            st_wo(i - 1)

    def mix1(j, _):
        c = rows(j, TF)
        bias = b1_s[:, c]
        g = [jax.nn.gelu(u + bias[:, (n % 2) * 256:(n % 2 + 1) * 256],
                         approximate=True)
             for n, u in enumerate(_strassen(ht, w1c, rows(j, 256)))]
        for n, a in enumerate(_strassen_lhs(*g)):
            g_s[n, :, rows(j, 256)] = _words(a.astype(bf16))
        return 0

    def layer(l, _):
        load_x(l, 0)
        load_x(l, 1)
        if l == 0:
            cp_wo.start()
            cp_x(2).start()
            cp_w1(0).start()
            cp_w1(1).start()
        with jax.named_scope("pro"):
            st_ln(0)
            k_s[:, TA:, :] = jnp.zeros((NB, PAD, 128), f32)
            v_s[:, TA:, :] = jnp.zeros((NB, PAD, 128), f32)
            attn_step(0, first=True)
            if l == 0:
                cp_wo.wait()
                jax.lax.fori_loop(0, NB // 2, perm_wo, 0)

        def attn_block(j, _):
            i = j + 1

            if l == 0:
                @pl.when(i + 1 < NA)
                def _():
                    @pl.when(i + 2 < NA)
                    def _():
                        cp_x(i + 2).start()
                    load_x(l, i + 1)
                stream(cp_w1, j)
                prep_w1(j)
            attn_step(i)
            return 0
        _loop("attn_block", NA - 1, attn_block)
        if l == 0:
            cp_w2(0).start()
            cp_w2(1).start()
        with jax.named_scope("epi"):
            attn_step(NA, last=True)
            st_h(NA - 1, 0)

        def mix1_(j, _):
            if l == 0:
                stream(cp_w2, j)
                prep_w2(j)
            return mix1(j, 0)
        _loop("mix1", F // TF, mix1_)

        def mix2(j, _):
            bias = b2_s[:, rows(j, TS)]
            for n, y in enumerate(_strassen(g_s, w2c, rows(j, 256))):
                y = y + bias[:, (n % 2) * 256:(n % 2 + 1) * 256]
                at = (rows(2 * j + n % 2, 256), rows(n // 2, HD))
                xn = xs[at] + y.T
                if l == 0:
                    xs[at] = xn
                else:
                    xin[at] = xn.astype(bf16)

            @pl.when(l == 1)
            def _():
                cp_out(j).start()
            return 0
        _loop("mix2", S // TS, mix2)
        return 0

    layer(0, 0)
    layer(1, 0)
    for j in range(S // TS):
        cp_out(j).wait()


@jax.jit
def pallas_interleave_layers__sliding_local_dilated__mixer_token_mlp__prompt_kernel(
    A_x: jax.Array,
    A_wqkv: jax.Array,
    A_wo: jax.Array,
    B_x: jax.Array,
    B_w1: jax.Array,
    B_b1: jax.Array,
    B_w2: jax.Array,
    B_b2: jax.Array,
):
    del B_x
    hbm = pl.BlockSpec(memory_space=pl.ANY)
    vmem = pl.BlockSpec(memory_space=pltpu.VMEM)
    out = pl.pallas_call(
        _kernel,
        in_specs=[hbm, hbm, hbm, hbm, vmem, hbm, vmem],
        out_specs=hbm,
        out_shape=jax.ShapeDtypeStruct((S, D), bf16),
        scratch_shapes=[
            pltpu.VMEM((S, D), bf16),
            pltpu.VMEM((D, 3 * D), bf16),
            pltpu.VMEM((D, D), bf16),
            pltpu.VMEM((3, S, TF), bf16),
            pltpu.VMEM((3, TF, S), bf16),
            pltpu.VMEM((7, S // 4, F // 2), jnp.uint32),
            pltpu.VMEM((7, F // 4, S // 2), jnp.uint32),
            pltpu.VMEM((S, D), f32),
            pltpu.VMEM((3, D + H, 128), jnp.uint32),
            pltpu.VMEM((2, D + H, 128), f32),
            pltpu.VMEM((TA, D), bf16),
            pltpu.VMEM((NB, TA, 128), f32),
            pltpu.VMEM((NB, PAD + TA, 128), f32),
            pltpu.VMEM((NB, PAD + TA, 128), f32),
            pltpu.VMEM((W, TA, 128), f32),
            pltpu.VMEM((TA, D), bf16),
            pltpu.VMEM((7, HD // 2, S // 2), jnp.uint32),
            pltpu.VMEM((7, HD // 2, F // 2), jnp.uint32),
            pltpu.VMEM((1, F), f32),
            pltpu.VMEM((1, S), f32),
            pltpu.SemaphoreType.DMA((13,)),
            pltpu.SemaphoreType.DMA((max(NA, S // TS),)),
        ],
        compiler_params=pltpu.CompilerParams(
            vmem_limit_bytes=124 * 1024 * 1024),
    )(A_x.reshape(S, D), A_wqkv, A_wo, B_w1, B_b1, B_w2,
      B_b2)
    return out.reshape(1, S, D)
```
